```python
import os as _os
_os.environ.setdefault('JAX_PLATFORMS', 'cpu')
import jax
import jax.numpy as jnp

def _softmax(x, axis=-1):
    return jax.nn.softmax(x, axis=axis)

def _gelu(x):
    return jax.nn.gelu(x, approximate=True)

def _silu(x):
    return jax.nn.silu(x)

def _sigmoid(x):
    return jax.nn.sigmoid(x)

def _layernorm(x, axis=-1, eps=1e-05):
    m = jnp.mean(x, axis=axis, keepdims=True)
    v = jnp.var(x, axis=axis, keepdims=True)
    return (x - m) / jnp.sqrt(v + eps)

def _scatter_add(tgt, idx, src, axis=0):
    return tgt.at[idx].add(src)

def _segment_sum(src, seg, n):
    return jax.ops.segment_sum(src, seg, n)

class _Rng:

    def __init__(self, key):
        self._k = key

    def _next(self):
        self._k, sub = jax.random.split(self._k)
        return sub

    def normal(self, shape):
        return jax.random.normal(self._next(), shape, dtype=jnp.bfloat16)

    def randint(self, lo, hi, shape):
        return jax.random.randint(self._next(), shape, lo, hi, dtype=jnp.int32)

    def uniform(self, shape, lo=0.0, hi=1.0):
        return jax.random.uniform(self._next(), shape, jnp.bfloat16, lo, hi)

    def permutation(self, n):
        return jax.random.permutation(self._next(), n)
kernel_name = 'adaLN_cond__mha_block__dense_activation_squared_relu__prompt'

def setup_inputs():
    _rng = _Rng(jax.random.key(int.from_bytes(__import__("os").urandom(4), "little")))
    _w = lambda a: (lambda t: t.astype(jnp.bfloat16) if jnp.issubdtype(t.dtype, jnp.floating) else t)(jnp.asarray(a))

    def _A_setup():
        B, S, D, H = (1, 2048, 512, 32)
        return {'x': _w((lambda *s: _rng.normal(s) * 0.05)(B, S, D)), 'wqkv': _w((lambda *s: _rng.normal(s) * 0.1)(D, 3 * D)), 'wo': _w((lambda *s: _rng.normal(s) * 0.05)(D, D))}
    _A_in = _A_setup()

    def _B_setup():
        B, S, D, F = (1, 2048, 512, 1792)
        return {'x': _w((lambda *s: _rng.normal(s) * 0.05)(B, S, D)), 'w1': _w((lambda *s: _rng.normal(s) * 0.05)(D, F)), 'b1': _w((lambda *s: _rng.normal(s) * 0.05)(F)), 'w2': _w((lambda *s: _rng.normal(s) * 0.05)(F, D)), 'b2': _w((lambda *s: _rng.normal(s) * 0.05)(D))}
    _B_in = _B_setup()
    return {'A_x': _A_in['x'], 'A_wqkv': _A_in['wqkv'], 'A_wo': _A_in['wo'], 'B_x': _B_in['x'], 'B_w1': _B_in['w1'], 'B_b1': _B_in['b1'], 'B_w2': _B_in['w2'], 'B_b2': _B_in['b2'], 'c': _w((lambda *s: _rng.normal(s) * 0.05)(1, 512) * 8.0), 'w_mod': _w((lambda *s: _rng.normal(s) * 0.05)(512, 6 * 512) * 512 ** (-0.5) * 8.0)}

def reference(A_x, A_wqkv, A_wo, B_x, B_w1, B_b1, B_w2, B_b2, c, w_mod):

    def _A_ref(x, wqkv, wo):
        B, S, D = x.shape
        H = 32
        Dh = D // H
        qkv = (lambda x, *d: x.transpose(*d))((x @ wqkv).reshape(B, S, 3, H, Dh), 2, 0, 3, 1, 4)
        q, k, v = (qkv[0], qkv[1], qkv[2])
        scores = jnp.einsum('bhqd,bhkd->bhqk', q, k) * Dh ** (-0.5)
        p = _softmax(scores, axis=-1)
        o = jnp.einsum('bhqk,bhkd->bhqd', p, v)
        return (lambda x, *d: x.transpose(*d))(o, 0, 2, 1, 3).reshape(B, S, D) @ wo

    def _B_ref(x, w1, b1, w2, b2):
        h = jnp.einsum('bsd,df->bsf', x, w1) + b1
        zero = jnp.zeros_like(h)
        r = jnp.where(h > zero, h, zero)
        h = r * r
        out = jnp.einsum('bsf,fd->bsd', h, w2) + b2
        return out
    x = A_x
    mod = (_silu(c) @ w_mod).reshape(c.shape[0], 6, 1, -1)
    sa, ca, ga, sb, cb, gb = (mod[:, 0].copy(), mod[:, 1].copy(), mod[:, 2].copy(), mod[:, 3].copy(), mod[:, 4].copy(), mod[:, 5].copy())
    h = _layernorm(x, axis=-1) * (1 + ca) + sa
    x = x + ga * _A_ref(h, A_wqkv, A_wo)
    h = _layernorm(x, axis=-1) * (1 + cb) + sb
    x = x + gb * _B_ref(h, B_w1, B_b1, B_w2, B_b2)
    return x
```

```python
import jax
import jax.numpy as jnp
from jax import lax
import jax.experimental.pallas as pl
import jax.experimental.pallas.tpu as pltpu

_LOG2E = 1.4426950408889634
_EPS = 1e-05


@jax.jit
def pallas_adaLN_cond__mha_block__dense_activation_squared_relu__prompt_kernel(
    A_x: jax.Array,
    A_wqkv: jax.Array,
    A_wo: jax.Array,
    B_x: jax.Array,
    B_w1: jax.Array,
    B_b1: jax.Array,
    B_w2: jax.Array,
    B_b2: jax.Array,
    c: jax.Array,
    w_mod: jax.Array,
):
    del B_x
    B, S, D = A_x.shape
    assert B == 1
    H = 32
    DH = D // H
    F = B_w1.shape[1]
    LANES = 128
    HPG = LANES // DH
    G = D // LANES
    TQ = 512
    CK = 128
    NQ = S // TQ
    NC = S // CK
    TR = 256
    q_scale = (DH ** -0.5) * _LOG2E

    f32 = jnp.float32
    bf16 = jnp.bfloat16

    def layernorm(x):
        m = jnp.mean(x, axis=-1, keepdims=True)
        xc = x - m
        v = jnp.mean(xc * xc, axis=-1, keepdims=True)
        return xc * lax.rsqrt(v + _EPS)

    def kernel(x_ref, wqkv_ref, wo_ref, w1_ref, b1_ref, w2_ref, b2_ref, c_ref,
               wmod_ref, o_ref,
               mod_ref, k_ref, qt_ref, vt_ref, ot_ref, s_ref):
        cc = c_ref[...].astype(f32)
        sc = (cc * jax.nn.sigmoid(cc)).astype(bf16)
        mod_ref[...] = jnp.dot(sc, wmod_ref[...], preferred_element_type=f32)

        sa = mod_ref[:, 0 * D:1 * D]
        ca = mod_ref[:, 1 * D:2 * D]

        for r in range(NQ):
            rows = pl.ds(r * TQ, TQ)
            xr = x_ref[rows, :].astype(f32)
            h = (layernorm(xr) * (1.0 + ca) + sa).astype(bf16)
            kk = jnp.dot(h, wqkv_ref[:, D:2 * D], preferred_element_type=f32)
            for g in range(G):
                k_ref[g, rows, :] = kk[:, g * LANES:(g + 1) * LANES].astype(bf16)
            qt = lax.dot_general(wqkv_ref[:, 0:D], h, (((0,), (1,)), ((), ())),
                                 preferred_element_type=f32)
            qt = (qt * q_scale).astype(bf16)
            for g in range(G):
                qt_ref[g, r] = qt[g * LANES:(g + 1) * LANES, :]
            vt = lax.dot_general(wqkv_ref[:, 2 * D:3 * D], h, (((0,), (1,)), ((), ())),
                                 preferred_element_type=f32)
            vt_ref[:, rows] = vt.astype(bf16)

        n_items = H * NQ

        def qmask(it):
            h = it // NQ
            j = it % NQ
            g = h // HPG
            hh = h % HPG
            q = qt_ref[g, j]
            row = lax.broadcasted_iota(jnp.int32, q.shape, 0)
            keep = (row >= hh * DH) & (row < hh * DH + DH)
            return g, jnp.where(keep, q, jnp.zeros_like(q))

        def red8(x, op):
            return op(x.reshape(CK // 8, 8, TQ), axis=0)

        g0, qm0 = qmask(0)
        mx0 = jnp.full((8, TQ), -jnp.inf, f32)
        for cidx in range(NC):
            rows = pl.ds(cidx * CK, CK)
            sn = jnp.dot(k_ref[g0, rows, :], qm0, preferred_element_type=f32)
            s_ref[rows, :] = sn
            mx0 = jnp.maximum(mx0, red8(sn, jnp.max))
        m0 = jnp.max(mx0, axis=0, keepdims=True)

        def body(it, m_cur):
            h = it // NQ
            j = it % NQ
            hrow = pl.ds(pl.multiple_of(h * DH, DH), DH)
            nxt = jnp.minimum(it + 1, n_items - 1)
            gn, qmn = qmask(nxt)
            mx = jnp.full((8, TQ), -jnp.inf, f32)
            l = jnp.zeros((8, TQ), f32)
            acc = jnp.zeros((DH, TQ), f32)
            for cidx in range(NC):
                rows = pl.ds(cidx * CK, CK)
                p = jnp.exp2(s_ref[rows, :] - m_cur)
                l = l + red8(p, jnp.sum)
                acc = acc + jnp.dot(vt_ref[hrow, rows], p.astype(bf16),
                                    preferred_element_type=f32)
                sn = jnp.dot(k_ref[gn, rows, :], qmn, preferred_element_type=f32)
                s_ref[rows, :] = sn
                mx = jnp.maximum(mx, red8(sn, jnp.max))
            lsum = jnp.sum(l, axis=0, keepdims=True)
            ot_ref[j, hrow, :] = (acc / lsum).astype(bf16)
            return jnp.max(mx, axis=0, keepdims=True)

        lax.fori_loop(0, n_items, body, m0)

        ga = mod_ref[:, 2 * D:3 * D]
        sb = mod_ref[:, 3 * D:4 * D]
        cb = mod_ref[:, 4 * D:5 * D]
        gb = mod_ref[:, 5 * D:6 * D]
        b1 = b1_ref[...].astype(f32)
        b2 = b2_ref[...].astype(f32)
        for r in range(S // TR):
            j = (r * TR) // TQ
            off = (r * TR) % TQ
            rows = pl.ds(r * TR, TR)
            attn = lax.dot_general(ot_ref[j, :, off:off + TR], wo_ref[...],
                                   (((0,), (0,)), ((), ())),
                                   preferred_element_type=f32)
            x1 = x_ref[rows, :].astype(f32) + ga * attn
            h2 = (layernorm(x1) * (1.0 + cb) + sb).astype(bf16)
            a = jnp.dot(h2, w1_ref[...], preferred_element_type=f32) + b1
            a = jnp.maximum(a, 0.0)
            a = (a * a).astype(bf16)
            y = jnp.dot(a, w2_ref[...], preferred_element_type=f32) + b2
            o_ref[rows, :] = (x1 + gb * y).astype(o_ref.dtype)

    out = pl.pallas_call(
        kernel,
        out_shape=jax.ShapeDtypeStruct((S, D), A_x.dtype),
        scratch_shapes=[
            pltpu.VMEM((1, 6 * D), f32),
            pltpu.VMEM((G, S, LANES), bf16),
            pltpu.VMEM((G, NQ, LANES, TQ), bf16),
            pltpu.VMEM((D, S), bf16),
            pltpu.VMEM((NQ, D, TQ), bf16),
            pltpu.VMEM((S, TQ), f32),
        ],
        compiler_params=pltpu.CompilerParams(vmem_limit_bytes=100 * 1024 * 1024),
    )(
        A_x.reshape(S, D), A_wqkv, A_wo, B_w1, B_b1.reshape(1, F), B_w2,
        B_b2.reshape(1, D), c, w_mod,
    )
    return out.reshape(B, S, D)
```

```python
import jax
import jax.numpy as jnp
from jax import lax
import jax.experimental.pallas as pl
import jax.experimental.pallas.tpu as pltpu

_LOG2E = 1.4426950408889634
_EPS = 1e-05


@jax.jit
def pallas_adaLN_cond__mha_block__dense_activation_squared_relu__prompt_kernel(
    A_x: jax.Array,
    A_wqkv: jax.Array,
    A_wo: jax.Array,
    B_x: jax.Array,
    B_w1: jax.Array,
    B_b1: jax.Array,
    B_w2: jax.Array,
    B_b2: jax.Array,
    c: jax.Array,
    w_mod: jax.Array,
):
    del B_x
    B, S, D = A_x.shape
    assert B == 1
    H = 32
    DH = D // H
    F = B_w1.shape[1]
    LANES = 128
    HPG = LANES // DH
    G = D // LANES
    TQ = 512
    CK = 128
    NQ = S // TQ
    NC = S // CK
    TR = 256
    q_scale = (DH ** -0.5) * _LOG2E

    f32 = jnp.float32
    bf16 = jnp.bfloat16

    def layernorm(x):
        m = jnp.mean(x, axis=-1, keepdims=True)
        xc = x - m
        v = jnp.mean(xc * xc, axis=-1, keepdims=True)
        return xc * lax.rsqrt(v + _EPS)

    def kernel(x_hbm, wqkv_hbm, wo_hbm, w1_hbm, b1_ref, w2_hbm, b2_ref, c_ref,
               wmod_hbm, o_hbm,
               x_ref, wqkv_ref, wo_ref, w1_ref, w2_ref, wmod_ref, o_ref,
               mod_ref, k_ref, qt_ref, vt_ref, ot_ref, s_ref, in_sems, out_sems):
        cp_wma = pltpu.make_async_copy(wmod_hbm.at[:, 0:2 * D], wmod_ref.at[:, 0:2 * D], in_sems.at[0])
        cp_x = [pltpu.make_async_copy(x_hbm.at[pl.ds(r * TQ, TQ), :], x_ref.at[pl.ds(r * TQ, TQ), :],
                                      in_sems.at[1 + r]) for r in range(NQ)]
        base = 1 + NQ
        cp_wk = pltpu.make_async_copy(wqkv_hbm.at[:, D:2 * D], wqkv_ref.at[:, D:2 * D], in_sems.at[base])
        cp_wq = pltpu.make_async_copy(wqkv_hbm.at[:, 0:D], wqkv_ref.at[:, 0:D], in_sems.at[base + 1])
        cp_wv = pltpu.make_async_copy(wqkv_hbm.at[:, 2 * D:3 * D], wqkv_ref.at[:, 2 * D:3 * D], in_sems.at[base + 2])
        cp_wmb = pltpu.make_async_copy(wmod_hbm.at[:, 2 * D:6 * D], wmod_ref.at[:, 2 * D:6 * D], in_sems.at[base + 3])
        cp_wo = pltpu.make_async_copy(wo_hbm, wo_ref, in_sems.at[base + 4])
        cp_w1 = pltpu.make_async_copy(w1_hbm, w1_ref, in_sems.at[base + 5])
        cp_w2 = pltpu.make_async_copy(w2_hbm, w2_ref, in_sems.at[base + 6])
        cp_wma.start()
        cp_x[0].start()
        cp_wk.start()
        cp_wq.start()
        cp_wv.start()
        for r in range(1, NQ):
            cp_x[r].start()
        cp_wmb.start()
        cp_wo.start()
        cp_w1.start()
        cp_w2.start()

        cc = c_ref[...].astype(f32)
        sc = (cc * jax.nn.sigmoid(cc)).astype(bf16)
        cp_wma.wait()
        mod_a = jnp.dot(sc, wmod_ref[:, 0:2 * D], preferred_element_type=f32)
        sa = mod_a[:, 0 * D:1 * D]
        ca = mod_a[:, 1 * D:2 * D]

        for r in range(NQ):
            rows = pl.ds(r * TQ, TQ)
            cp_x[r].wait()
            xr = x_ref[rows, :].astype(f32)
            h = (layernorm(xr) * (1.0 + ca) + sa).astype(bf16)
            if r == 0:
                cp_wk.wait()
            kk = jnp.dot(h, wqkv_ref[:, D:2 * D], preferred_element_type=f32)
            for g in range(G):
                k_ref[g, rows, :] = kk[:, g * LANES:(g + 1) * LANES].astype(bf16)
            if r == 0:
                cp_wq.wait()
            qt = lax.dot_general(wqkv_ref[:, 0:D], h, (((0,), (1,)), ((), ())),
                                 preferred_element_type=f32)
            qt = (qt * q_scale).astype(bf16)
            for g in range(G):
                qt_ref[g, r] = qt[g * LANES:(g + 1) * LANES, :]
            if r == 0:
                cp_wv.wait()
            vt = lax.dot_general(wqkv_ref[:, 2 * D:3 * D], h, (((0,), (1,)), ((), ())),
                                 preferred_element_type=f32)
            vt_ref[:, rows] = vt.astype(bf16)

        n_items = H * NQ

        def qmask(it):
            h = it // NQ
            j = it % NQ
            g = h // HPG
            hh = h % HPG
            q = qt_ref[g, j]
            row = lax.broadcasted_iota(jnp.int32, q.shape, 0)
            keep = (row >= hh * DH) & (row < hh * DH + DH)
            return g, jnp.where(keep, q, jnp.zeros_like(q))

        def red8(x, op):
            return op(x.reshape(CK // 8, 8, TQ), axis=0)

        g0, qm0 = qmask(0)
        mx0 = jnp.full((8, TQ), -jnp.inf, f32)
        for cidx in range(NC):
            rows = pl.ds(cidx * CK, CK)
            sn = jnp.dot(k_ref[g0, rows, :], qm0, preferred_element_type=f32)
            s_ref[rows, :] = sn
            mx0 = jnp.maximum(mx0, red8(sn, jnp.max))
        m0 = jnp.max(mx0, axis=0, keepdims=True)

        def body(it, m_cur):
            h = it // NQ
            j = it % NQ
            hrow = pl.ds(pl.multiple_of(h * DH, DH), DH)
            nxt = jnp.minimum(it + 1, n_items - 1)
            gn, qmn = qmask(nxt)
            mx = jnp.full((8, TQ), -jnp.inf, f32)
            l = jnp.zeros((8, TQ), f32)
            acc = jnp.zeros((DH, TQ), f32)
            for cidx in range(NC):
                rows = pl.ds(cidx * CK, CK)
                p = jnp.exp2(s_ref[rows, :] - m_cur)
                l = l + red8(p, jnp.sum)
                acc = acc + jnp.dot(vt_ref[hrow, rows], p.astype(bf16),
                                    preferred_element_type=f32)
                sn = jnp.dot(k_ref[gn, rows, :], qmn, preferred_element_type=f32)
                s_ref[rows, :] = sn
                mx = jnp.maximum(mx, red8(sn, jnp.max))
            lsum = jnp.sum(l, axis=0, keepdims=True)
            ot_ref[j, hrow, :] = (acc / lsum).astype(bf16)
            return jnp.max(mx, axis=0, keepdims=True)

        lax.fori_loop(0, n_items, body, m0)

        cp_wmb.wait()
        cp_wo.wait()
        cp_w1.wait()
        cp_w2.wait()
        mod_b = jnp.dot(sc, wmod_ref[:, 2 * D:6 * D], preferred_element_type=f32)
        ga = mod_b[:, 0 * D:1 * D]
        sb = mod_b[:, 1 * D:2 * D]
        cb = mod_b[:, 2 * D:3 * D]
        gb = mod_b[:, 3 * D:4 * D]
        cp_out = [pltpu.make_async_copy(o_ref.at[pl.ds(r * TR, TR), :], o_hbm.at[pl.ds(r * TR, TR), :],
                                        out_sems.at[r]) for r in range(S // TR)]
        b1 = b1_ref[...].astype(f32)
        b2 = b2_ref[...].astype(f32)
        for r in range(S // TR):
            j = (r * TR) // TQ
            off = (r * TR) % TQ
            rows = pl.ds(r * TR, TR)
            attn = lax.dot_general(ot_ref[j, :, off:off + TR], wo_ref[...],
                                   (((0,), (0,)), ((), ())),
                                   preferred_element_type=f32)
            x1 = x_ref[rows, :].astype(f32) + ga * attn
            h2 = (layernorm(x1) * (1.0 + cb) + sb).astype(bf16)
            a = jnp.dot(h2, w1_ref[...], preferred_element_type=f32) + b1
            a = jnp.maximum(a, 0.0)
            a = (a * a).astype(bf16)
            y = jnp.dot(a, w2_ref[...], preferred_element_type=f32) + b2
            o_ref[rows, :] = (x1 + gb * y).astype(o_ref.dtype)
            cp_out[r].start()
        for r in range(S // TR):
            cp_out[r].wait()

    any_spec = pl.BlockSpec(memory_space=pl.ANY)
    vmem_spec = pl.BlockSpec(memory_space=pltpu.VMEM)
    out = pl.pallas_call(
        kernel,
        out_shape=jax.ShapeDtypeStruct((S, D), A_x.dtype),
        in_specs=[any_spec, any_spec, any_spec, any_spec, vmem_spec, any_spec,
                  vmem_spec, vmem_spec, any_spec],
        out_specs=any_spec,
        scratch_shapes=[
            pltpu.VMEM((S, D), bf16),
            pltpu.VMEM((D, 3 * D), bf16),
            pltpu.VMEM((D, D), bf16),
            pltpu.VMEM((D, F), bf16),
            pltpu.VMEM((F, D), bf16),
            pltpu.VMEM((D, 6 * D), bf16),
            pltpu.VMEM((S, D), bf16),
            pltpu.VMEM((1, 6 * D), f32),
            pltpu.VMEM((G, S, LANES), bf16),
            pltpu.VMEM((G, NQ, LANES, TQ), bf16),
            pltpu.VMEM((D, S), bf16),
            pltpu.VMEM((NQ, D, TQ), bf16),
            pltpu.VMEM((S, TQ), f32),
            pltpu.SemaphoreType.DMA((1 + NQ + 7,)),
            pltpu.SemaphoreType.DMA((S // TR,)),
        ],
        compiler_params=pltpu.CompilerParams(vmem_limit_bytes=100 * 1024 * 1024),
    )(
        A_x.reshape(S, D), A_wqkv, A_wo, B_w1, B_b1.reshape(1, F), B_w2,
        B_b2.reshape(1, D), c, w_mod,
    )
    return out.reshape(B, S, D)
```

```python
import jax
import jax.numpy as jnp
from jax import lax
import jax.experimental.pallas as pl
import jax.experimental.pallas.tpu as pltpu

_LOG2E = 1.4426950408889634
_EPS = 1e-05


@jax.jit
def pallas_adaLN_cond__mha_block__dense_activation_squared_relu__prompt_kernel(
    A_x: jax.Array,
    A_wqkv: jax.Array,
    A_wo: jax.Array,
    B_x: jax.Array,
    B_w1: jax.Array,
    B_b1: jax.Array,
    B_w2: jax.Array,
    B_b2: jax.Array,
    c: jax.Array,
    w_mod: jax.Array,
):
    del B_x
    B, S, D = A_x.shape
    assert B == 1
    H = 32
    DH = D // H
    F = B_w1.shape[1]
    LANES = 128
    HPG = LANES // DH
    G = D // LANES
    TQ = 512
    CK = 128
    NQ = S // TQ
    NC = S // CK
    TR = TQ
    q_scale = (DH ** -0.5) * _LOG2E

    f32 = jnp.float32
    bf16 = jnp.bfloat16

    def layernorm(x):
        m = jnp.mean(x, axis=-1, keepdims=True)
        xc = x - m
        v = jnp.mean(xc * xc, axis=-1, keepdims=True)
        return xc * lax.rsqrt(v + _EPS)

    def kernel(x_hbm, wqkv_hbm, wo_hbm, w1_hbm, b1_ref, w2_hbm, b2_ref, c_ref,
               wmod_hbm, o_hbm,
               x_ref, wqkv_ref, wo_ref, w1_ref, w2_ref, wmod_ref, o_ref,
               mod_ref, k_ref, qt_ref, vt_ref, ot_ref, s_ref, in_sems, out_sems):
        cp_wma = pltpu.make_async_copy(wmod_hbm.at[:, 0:2 * D], wmod_ref.at[:, 0:2 * D], in_sems.at[0])
        cp_x = [pltpu.make_async_copy(x_hbm.at[pl.ds(r * TQ, TQ), :], x_ref.at[pl.ds(r * TQ, TQ), :],
                                      in_sems.at[1 + r]) for r in range(NQ)]
        base = 1 + NQ
        cp_wk = pltpu.make_async_copy(wqkv_hbm.at[:, D:2 * D], wqkv_ref.at[:, D:2 * D], in_sems.at[base])
        cp_wq = pltpu.make_async_copy(wqkv_hbm.at[:, 0:D], wqkv_ref.at[:, 0:D], in_sems.at[base + 1])
        cp_wv = pltpu.make_async_copy(wqkv_hbm.at[:, 2 * D:3 * D], wqkv_ref.at[:, 2 * D:3 * D], in_sems.at[base + 2])
        cp_wmb = pltpu.make_async_copy(wmod_hbm.at[:, 2 * D:6 * D], wmod_ref.at[:, 2 * D:6 * D], in_sems.at[base + 3])
        cp_wo = pltpu.make_async_copy(wo_hbm, wo_ref, in_sems.at[base + 4])
        cp_w1 = pltpu.make_async_copy(w1_hbm, w1_ref, in_sems.at[base + 5])
        cp_w2 = pltpu.make_async_copy(w2_hbm, w2_ref, in_sems.at[base + 6])
        cp_wma.start()
        cp_x[0].start()
        cp_wk.start()
        cp_wq.start()
        cp_wv.start()
        for r in range(1, NQ):
            cp_x[r].start()

        cc = c_ref[...].astype(f32)
        sc = (cc * jax.nn.sigmoid(cc)).astype(bf16)
        cp_wma.wait()
        mod_a = jnp.dot(sc, wmod_ref[:, 0:2 * D], preferred_element_type=f32)
        sa = mod_a[:, 0 * D:1 * D]
        ca = mod_a[:, 1 * D:2 * D]

        cp_wk.wait()
        cp_wq.wait()
        cp_wv.wait()

        def proj_body(r, carry):
            rows = pl.ds(pl.multiple_of(r * TQ, TQ), TQ)
            pltpu.make_async_copy(x_hbm.at[rows, :], x_ref.at[rows, :], in_sems.at[1 + r]).wait()
            xr = x_ref[rows, :].astype(f32)
            h = (layernorm(xr) * (1.0 + ca) + sa).astype(bf16)
            kk = jnp.dot(h, wqkv_ref[:, D:2 * D], preferred_element_type=f32)
            for g in range(G):
                k_ref[g, rows, :] = kk[:, g * LANES:(g + 1) * LANES].astype(bf16)
            qt = lax.dot_general(wqkv_ref[:, 0:D], h, (((0,), (1,)), ((), ())),
                                 preferred_element_type=f32)
            qt = (qt * q_scale).astype(bf16)
            for g in range(G):
                qt_ref[g, r] = qt[g * LANES:(g + 1) * LANES, :]
            vt = lax.dot_general(wqkv_ref[:, 2 * D:3 * D], h, (((0,), (1,)), ((), ())),
                                 preferred_element_type=f32)
            vt_ref[:, rows] = vt.astype(bf16)
            return carry

        lax.fori_loop(0, NQ, proj_body, 0)

        cp_wmb.start()
        cp_wo.start()
        cp_w1.start()
        cp_w2.start()

        n_items = H * NQ

        def qmask(it):
            h = it // NQ
            j = it % NQ
            g = h // HPG
            hh = h % HPG
            q = qt_ref[g, j]
            row = lax.broadcasted_iota(jnp.int32, q.shape, 0)
            keep = (row >= hh * DH) & (row < hh * DH + DH)
            return g, jnp.where(keep, q, jnp.zeros_like(q))

        def red8(x, op):
            return op(x.reshape(CK // 8, 8, TQ), axis=0)

        g0, qm0 = qmask(0)
        mx0 = jnp.full((8, TQ), -jnp.inf, f32)
        for cidx in range(NC):
            rows = pl.ds(cidx * CK, CK)
            sn = jnp.dot(k_ref[g0, rows, :], qm0, preferred_element_type=f32)
            s_ref[rows, :] = sn
            mx0 = jnp.maximum(mx0, red8(sn, jnp.max))
        m0 = jnp.max(mx0, axis=0, keepdims=True)

        def body(it, m_cur):
            h = it // NQ
            j = it % NQ
            hrow = pl.ds(pl.multiple_of(h * DH, DH), DH)
            nxt = jnp.minimum(it + 1, n_items - 1)
            gn, qmn = qmask(nxt)
            mx = jnp.full((8, TQ), -jnp.inf, f32)
            l = jnp.zeros((8, TQ), f32)
            acc = jnp.zeros((DH, TQ), f32)
            for cidx in range(NC):
                rows = pl.ds(cidx * CK, CK)
                p = jnp.exp2(s_ref[rows, :] - m_cur)
                l = l + red8(p, jnp.sum)
                acc = acc + jnp.dot(vt_ref[hrow, rows], p.astype(bf16),
                                    preferred_element_type=f32)
                sn = jnp.dot(k_ref[gn, rows, :], qmn, preferred_element_type=f32)
                s_ref[rows, :] = sn
                mx = jnp.maximum(mx, red8(sn, jnp.max))
            lsum = jnp.sum(l, axis=0, keepdims=True)
            ot_ref[j, hrow, :] = (acc / lsum).astype(bf16)
            return jnp.max(mx, axis=0, keepdims=True)

        lax.fori_loop(0, n_items, body, m0)

        cp_wmb.wait()
        cp_wo.wait()
        cp_w1.wait()
        cp_w2.wait()
        mod_b = jnp.dot(sc, wmod_ref[:, 2 * D:6 * D], preferred_element_type=f32)
        ga = mod_b[:, 0 * D:1 * D]
        sb = mod_b[:, 1 * D:2 * D]
        cb = mod_b[:, 2 * D:3 * D]
        gb = mod_b[:, 3 * D:4 * D]
        b1 = b1_ref[...].astype(f32)
        b2 = b2_ref[...].astype(f32)

        def mlp_body(r, carry):
            rows = pl.ds(pl.multiple_of(r * TR, TR), TR)
            attn = lax.dot_general(ot_ref[r], wo_ref[...],
                                   (((0,), (0,)), ((), ())),
                                   preferred_element_type=f32)
            x1 = x_ref[rows, :].astype(f32) + ga * attn
            h2 = (layernorm(x1) * (1.0 + cb) + sb).astype(bf16)
            a = jnp.dot(h2, w1_ref[...], preferred_element_type=f32) + b1
            a = jnp.maximum(a, 0.0)
            a = (a * a).astype(bf16)
            y = jnp.dot(a, w2_ref[...], preferred_element_type=f32) + b2
            o_ref[rows, :] = (x1 + gb * y).astype(o_ref.dtype)
            pltpu.make_async_copy(o_ref.at[rows, :], o_hbm.at[rows, :], out_sems.at[r]).start()
            return carry

        lax.fori_loop(0, S // TR, mlp_body, 0)
        for r in range(S // TR):
            pltpu.make_async_copy(o_ref.at[pl.ds(r * TR, TR), :], o_hbm.at[pl.ds(r * TR, TR), :],
                                  out_sems.at[r]).wait()

    any_spec = pl.BlockSpec(memory_space=pl.ANY)
    vmem_spec = pl.BlockSpec(memory_space=pltpu.VMEM)
    out = pl.pallas_call(
        kernel,
        out_shape=jax.ShapeDtypeStruct((S, D), A_x.dtype),
        in_specs=[any_spec, any_spec, any_spec, any_spec, vmem_spec, any_spec,
                  vmem_spec, vmem_spec, any_spec],
        out_specs=any_spec,
        scratch_shapes=[
            pltpu.VMEM((S, D), bf16),
            pltpu.VMEM((D, 3 * D), bf16),
            pltpu.VMEM((D, D), bf16),
            pltpu.VMEM((D, F), bf16),
            pltpu.VMEM((F, D), bf16),
            pltpu.VMEM((D, 6 * D), bf16),
            pltpu.VMEM((S, D), bf16),
            pltpu.VMEM((1, 6 * D), f32),
            pltpu.VMEM((G, S, LANES), bf16),
            pltpu.VMEM((G, NQ, LANES, TQ), bf16),
            pltpu.VMEM((D, S), bf16),
            pltpu.VMEM((NQ, D, TQ), bf16),
            pltpu.VMEM((S, TQ), f32),
            pltpu.SemaphoreType.DMA((1 + NQ + 7,)),
            pltpu.SemaphoreType.DMA((S // TR,)),
        ],
        compiler_params=pltpu.CompilerParams(vmem_limit_bytes=100 * 1024 * 1024),
    )(
        A_x.reshape(S, D), A_wqkv, A_wo, B_w1, B_b1.reshape(1, F), B_w2,
        B_b2.reshape(1, D), c, w_mod,
    )
    return out.reshape(B, S, D)
```

```python
import jax
import jax.numpy as jnp
from jax import lax
import jax.experimental.pallas as pl
import jax.experimental.pallas.tpu as pltpu

_LOG2E = 1.4426950408889634
_EPS = 1e-05


@jax.jit
def pallas_adaLN_cond__mha_block__dense_activation_squared_relu__prompt_kernel(
    A_x: jax.Array,
    A_wqkv: jax.Array,
    A_wo: jax.Array,
    B_x: jax.Array,
    B_w1: jax.Array,
    B_b1: jax.Array,
    B_w2: jax.Array,
    B_b2: jax.Array,
    c: jax.Array,
    w_mod: jax.Array,
):
    del B_x
    B, S, D = A_x.shape
    assert B == 1
    H = 32
    DH = D // H
    F = B_w1.shape[1]
    LANES = 128
    HPG = LANES // DH
    G = D // LANES
    TQ = 512
    CK = 128
    NQ = S // TQ
    NC = S // CK
    TR = TQ
    q_scale = (DH ** -0.5) * _LOG2E

    f32 = jnp.float32
    bf16 = jnp.bfloat16

    def layernorm(x):
        m = jnp.mean(x, axis=-1, keepdims=True)
        xc = x - m
        v = jnp.mean(xc * xc, axis=-1, keepdims=True)
        return xc * lax.rsqrt(v + _EPS)

    def kernel(x_hbm, wqkv_hbm, wo_hbm, w1_hbm, b1_ref, w2_hbm, b2_ref, c_ref,
               wmod_hbm, o_hbm,
               x_ref, wqkv_ref, wo_ref, w1_ref, w2_ref, wmod_ref, o_ref,
               qm_ref, k_ref, qt_ref, vt_ref, ot_ref, s_ref, in_sems, out_sems):
        cp_wma = pltpu.make_async_copy(wmod_hbm.at[:, 0:2 * D], wmod_ref.at[:, 0:2 * D], in_sems.at[0])
        cp_x = [pltpu.make_async_copy(x_hbm.at[pl.ds(r * TQ, TQ), :], x_ref.at[pl.ds(r * TQ, TQ), :],
                                      in_sems.at[1 + r]) for r in range(NQ)]
        base = 1 + NQ
        cp_wk = pltpu.make_async_copy(wqkv_hbm.at[:, D:2 * D], wqkv_ref.at[:, D:2 * D], in_sems.at[base])
        cp_wq = pltpu.make_async_copy(wqkv_hbm.at[:, 0:D], wqkv_ref.at[:, 0:D], in_sems.at[base + 1])
        cp_wv = pltpu.make_async_copy(wqkv_hbm.at[:, 2 * D:3 * D], wqkv_ref.at[:, 2 * D:3 * D], in_sems.at[base + 2])
        cp_wmb = pltpu.make_async_copy(wmod_hbm.at[:, 2 * D:6 * D], wmod_ref.at[:, 2 * D:6 * D], in_sems.at[base + 3])
        cp_wo = pltpu.make_async_copy(wo_hbm, wo_ref, in_sems.at[base + 4])
        cp_w1 = pltpu.make_async_copy(w1_hbm, w1_ref, in_sems.at[base + 5])
        cp_w2 = pltpu.make_async_copy(w2_hbm, w2_ref, in_sems.at[base + 6])
        cp_wma.start()
        cp_x[0].start()
        cp_wk.start()
        cp_wq.start()
        cp_wv.start()
        for r in range(1, NQ):
            cp_x[r].start()

        cc = c_ref[...].astype(f32)
        sc = (cc * jax.nn.sigmoid(cc)).astype(bf16)
        cp_wma.wait()
        mod_a = jnp.dot(sc, wmod_ref[:, 0:2 * D], preferred_element_type=f32)
        sa = mod_a[:, 0 * D:1 * D]
        ca = mod_a[:, 1 * D:2 * D]

        cp_wk.wait()
        cp_wq.wait()
        cp_wv.wait()

        def proj_body(r, carry):
            rows = pl.ds(pl.multiple_of(r * TQ, TQ), TQ)
            pltpu.make_async_copy(x_hbm.at[rows, :], x_ref.at[rows, :], in_sems.at[1 + r]).wait()
            xr = x_ref[rows, :].astype(f32)
            h = (layernorm(xr) * (1.0 + ca) + sa).astype(bf16)
            kk = jnp.dot(h, wqkv_ref[:, D:2 * D], preferred_element_type=f32)
            for g in range(G):
                k_ref[g, rows, :] = kk[:, g * LANES:(g + 1) * LANES].astype(bf16)
            qt = lax.dot_general(wqkv_ref[:, 0:D], h, (((0,), (1,)), ((), ())),
                                 preferred_element_type=f32)
            qt = (qt * q_scale).astype(bf16)
            for g in range(G):
                qt_ref[g, r] = qt[g * LANES:(g + 1) * LANES, :]
            vt = lax.dot_general(wqkv_ref[:, 2 * D:3 * D], h, (((0,), (1,)), ((), ())),
                                 preferred_element_type=f32)
            vt_ref[:, rows] = vt.astype(bf16)
            return carry

        lax.fori_loop(0, NQ, proj_body, 0)

        cp_wmb.start()
        cp_wo.start()
        cp_w1.start()
        cp_w2.start()

        n_items = H * NQ

        def qmask(it):
            h = it // NQ
            j = it % NQ
            g = h // HPG
            hh = h % HPG
            q = qt_ref[g, j]
            row = lax.broadcasted_iota(jnp.int32, q.shape, 0)
            keep = (row >= hh * DH) & (row < hh * DH + DH)
            return g, jnp.where(keep, q, jnp.zeros_like(q))

        def red8(x, op):
            return op(x.reshape(CK // 8, 8, TQ), axis=0)

        g0, qm0 = qmask(0)
        mx0 = jnp.full((8, TQ), -jnp.inf, f32)
        for cidx in range(NC):
            rows = pl.ds(cidx * CK, CK)
            sn = jnp.dot(k_ref[g0, rows, :], qm0, preferred_element_type=f32)
            s_ref[rows, :] = sn
            mx0 = jnp.maximum(mx0, red8(sn, jnp.max))
        m0 = jnp.max(mx0, axis=0, keepdims=True)
        qm_ref[1] = qmask(1)[1]

        def body(it, m_cur):
            h = it // NQ
            j = it % NQ
            hrow = pl.ds(pl.multiple_of(h * DH, DH), DH)
            nxt = jnp.minimum(it + 1, n_items - 1)
            gn = (nxt // NQ) // HPG
            qmn = qm_ref[(it + 1) % 2]
            mx = jnp.full((8, TQ), -jnp.inf, f32)
            l = jnp.zeros((8, TQ), f32)
            acc = jnp.zeros((DH, TQ), f32)
            for cidx in range(NC):
                rows = pl.ds(cidx * CK, CK)
                p = jnp.exp2(s_ref[rows, :] - m_cur)
                l = l + red8(p, jnp.sum)
                acc = acc + jnp.dot(vt_ref[hrow, rows], p.astype(bf16),
                                    preferred_element_type=f32)
                sn = jnp.dot(k_ref[gn, rows, :], qmn, preferred_element_type=f32)
                s_ref[rows, :] = sn
                mx = jnp.maximum(mx, red8(sn, jnp.max))
            lsum = jnp.sum(l, axis=0, keepdims=True)
            ot_ref[j, hrow, :] = (acc / lsum).astype(bf16)
            qm_ref[it % 2] = qmask(jnp.minimum(it + 2, n_items - 1))[1]
            return jnp.max(mx, axis=0, keepdims=True)

        lax.fori_loop(0, n_items, body, m0)

        cp_wmb.wait()
        cp_wo.wait()
        cp_w1.wait()
        cp_w2.wait()
        mod_b = jnp.dot(sc, wmod_ref[:, 2 * D:6 * D], preferred_element_type=f32)
        ga = mod_b[:, 0 * D:1 * D]
        sb = mod_b[:, 1 * D:2 * D]
        cb = mod_b[:, 2 * D:3 * D]
        gb = mod_b[:, 3 * D:4 * D]
        b1 = b1_ref[...].astype(f32).reshape(1, F)
        b2 = b2_ref[...].astype(f32).reshape(1, D)

        def mlp_body(r, carry):
            rows = pl.ds(pl.multiple_of(r * TR, TR), TR)
            attn = lax.dot_general(ot_ref[r], wo_ref[...],
                                   (((0,), (0,)), ((), ())),
                                   preferred_element_type=f32)
            x1 = x_ref[rows, :].astype(f32) + ga * attn
            h2 = (layernorm(x1) * (1.0 + cb) + sb).astype(bf16)
            a = jnp.dot(h2, w1_ref[...], preferred_element_type=f32) + b1
            a = jnp.maximum(a, 0.0)
            a = (a * a).astype(bf16)
            y = jnp.dot(a, w2_ref[...], preferred_element_type=f32) + b2
            o_ref[rows, :] = (x1 + gb * y).astype(o_ref.dtype)
            pltpu.make_async_copy(o_ref.at[rows, :], o_hbm.at[rows, :], out_sems.at[r]).start()
            return carry

        lax.fori_loop(0, S // TR, mlp_body, 0)
        for r in range(S // TR):
            pltpu.make_async_copy(o_ref.at[pl.ds(r * TR, TR), :], o_hbm.at[pl.ds(r * TR, TR), :],
                                  out_sems.at[r]).wait()

    any_spec = pl.BlockSpec(memory_space=pl.ANY)
    vmem_spec = pl.BlockSpec(memory_space=pltpu.VMEM)
    out = pl.pallas_call(
        kernel,
        out_shape=jax.ShapeDtypeStruct((S, D), A_x.dtype),
        in_specs=[any_spec, any_spec, any_spec, any_spec, vmem_spec, any_spec,
                  vmem_spec, vmem_spec, any_spec],
        out_specs=any_spec,
        scratch_shapes=[
            pltpu.VMEM((S, D), bf16),
            pltpu.VMEM((D, 3 * D), bf16),
            pltpu.VMEM((D, D), bf16),
            pltpu.VMEM((D, F), bf16),
            pltpu.VMEM((F, D), bf16),
            pltpu.VMEM((D, 6 * D), bf16),
            pltpu.VMEM((S, D), bf16),
            pltpu.VMEM((2, LANES, TQ), bf16),
            pltpu.VMEM((G, S, LANES), bf16),
            pltpu.VMEM((G, NQ, LANES, TQ), bf16),
            pltpu.VMEM((D, S), bf16),
            pltpu.VMEM((NQ, D, TQ), bf16),
            pltpu.VMEM((S, TQ), f32),
            pltpu.SemaphoreType.DMA((1 + NQ + 7,)),
            pltpu.SemaphoreType.DMA((S // TR,)),
        ],
        compiler_params=pltpu.CompilerParams(vmem_limit_bytes=100 * 1024 * 1024),
    )(
        A_x.reshape(S, D), A_wqkv, A_wo, B_w1, B_b1, B_w2,
        B_b2, c, w_mod,
    )
    return out.reshape(B, S, D)
```

```python
import jax
import jax.numpy as jnp
from jax import lax
import jax.experimental.pallas as pl
import jax.experimental.pallas.tpu as pltpu

_LOG2E = 1.4426950408889634
_EPS = 1e-05


@jax.jit
def pallas_adaLN_cond__mha_block__dense_activation_squared_relu__prompt_kernel(
    A_x: jax.Array,
    A_wqkv: jax.Array,
    A_wo: jax.Array,
    B_x: jax.Array,
    B_w1: jax.Array,
    B_b1: jax.Array,
    B_w2: jax.Array,
    B_b2: jax.Array,
    c: jax.Array,
    w_mod: jax.Array,
):
    del B_x
    B, S, D = A_x.shape
    assert B == 1
    H = 32
    DH = D // H
    F = B_w1.shape[1]
    LANES = 128
    HPG = LANES // DH
    G = D // LANES
    TQ = 512
    CK = 128
    NQ = S // TQ
    NC = S // CK
    TR = TQ
    q_scale = (DH ** -0.5) * _LOG2E

    f32 = jnp.float32
    bf16 = jnp.bfloat16

    def layernorm(x):
        m = jnp.mean(x, axis=-1, keepdims=True)
        xc = x - m
        v = jnp.mean(xc * xc, axis=-1, keepdims=True)
        return xc * lax.rsqrt(v + _EPS)

    def kernel(x_hbm, wqkv_hbm, wo_hbm, w1_hbm, b1_ref, w2_hbm, b2_ref, c_ref,
               wmod_hbm, o_hbm,
               x_ref, wqkv_ref, wo_ref, w1_ref, w2_ref, wmod_ref, o_ref,
               qm_ref, k_ref, qt_ref, vt_ref, ot_ref, s_ref, in_sems, out_sems):
        cp_wma = pltpu.make_async_copy(wmod_hbm.at[:, 0:2 * D], wmod_ref.at[:, 0:2 * D], in_sems.at[0])
        cp_x = [pltpu.make_async_copy(x_hbm.at[pl.ds(r * TQ, TQ), :], x_ref.at[pl.ds(r * TQ, TQ), :],
                                      in_sems.at[1 + r]) for r in range(NQ)]
        base = 1 + NQ
        cp_wk = pltpu.make_async_copy(wqkv_hbm.at[:, D:2 * D], wqkv_ref.at[:, D:2 * D], in_sems.at[base])
        cp_wq = pltpu.make_async_copy(wqkv_hbm.at[:, 0:D], wqkv_ref.at[:, 0:D], in_sems.at[base + 1])
        cp_wv = pltpu.make_async_copy(wqkv_hbm.at[:, 2 * D:3 * D], wqkv_ref.at[:, 2 * D:3 * D], in_sems.at[base + 2])
        cp_wmb = pltpu.make_async_copy(wmod_hbm.at[:, 2 * D:6 * D], wmod_ref.at[:, 2 * D:6 * D], in_sems.at[base + 3])
        cp_wo = pltpu.make_async_copy(wo_hbm, wo_ref, in_sems.at[base + 4])
        cp_w1 = pltpu.make_async_copy(w1_hbm, w1_ref, in_sems.at[base + 5])
        cp_w2 = pltpu.make_async_copy(w2_hbm, w2_ref, in_sems.at[base + 6])
        cp_wma.start()
        cp_x[0].start()
        cp_wk.start()
        cp_wq.start()
        cp_wv.start()
        for r in range(1, NQ):
            cp_x[r].start()

        cc = c_ref[...].astype(f32)
        sc = (cc * jax.nn.sigmoid(cc)).astype(bf16)
        cp_wma.wait()
        mod_a = jnp.dot(sc, wmod_ref[:, 0:2 * D], preferred_element_type=f32)
        sa = mod_a[:, 0 * D:1 * D]
        ca = mod_a[:, 1 * D:2 * D]

        cp_wk.wait()
        cp_wq.wait()
        cp_wv.wait()

        def proj_body(r, carry):
            rows = pl.ds(pl.multiple_of(r * TQ, TQ), TQ)
            pltpu.make_async_copy(x_hbm.at[rows, :], x_ref.at[rows, :], in_sems.at[1 + r]).wait()
            xr = x_ref[rows, :].astype(f32)
            h = (layernorm(xr) * (1.0 + ca) + sa).astype(bf16)
            kk = jnp.dot(h, wqkv_ref[:, D:2 * D], preferred_element_type=f32)
            for g in range(G):
                k_ref[g, rows, :] = kk[:, g * LANES:(g + 1) * LANES].astype(bf16)
            qt = lax.dot_general(wqkv_ref[:, 0:D], h, (((0,), (1,)), ((), ())),
                                 preferred_element_type=f32)
            qt = (qt * q_scale).astype(bf16)
            for g in range(G):
                qt_ref[g, r] = qt[g * LANES:(g + 1) * LANES, :]
            vt = lax.dot_general(wqkv_ref[:, 2 * D:3 * D], h, (((0,), (1,)), ((), ())),
                                 preferred_element_type=f32)
            vt_ref[:, rows] = vt.astype(bf16)
            return carry

        lax.fori_loop(0, NQ, proj_body, 0)

        cp_wmb.start()
        cp_wo.start()
        cp_w1.start()
        cp_w2.start()

        n_items = H * NQ

        def qmask(it):
            h = it // NQ
            j = it % NQ
            g = h // HPG
            hh = h % HPG
            q = qt_ref[g, j]
            row = lax.broadcasted_iota(jnp.int32, q.shape, 0)
            keep = (row >= hh * DH) & (row < hh * DH + DH)
            return g, jnp.where(keep, q, jnp.zeros_like(q))

        def red8(x, op):
            return op(x.reshape(CK // 8, 8, TQ), axis=0)

        g0, qm0 = qmask(0)
        mx0 = jnp.full((8, TQ), -jnp.inf, f32)
        for cidx in range(NC):
            rows = pl.ds(cidx * CK, CK)
            sn = jnp.dot(k_ref[g0, rows, :], qm0, preferred_element_type=f32)
            s_ref[rows, :] = sn
            mx0 = jnp.maximum(mx0, red8(sn, jnp.max))
        m0 = jnp.max(mx0, axis=0, keepdims=True)
        qm_ref[1] = qmask(1)[1]

        def attend(it, m_cur, with_next):
            h = it // NQ
            j = it % NQ
            hrow = pl.ds(pl.multiple_of(h * DH, DH), DH)
            if with_next:
                gn = ((it + 1) // NQ) // HPG
                qmn = qm_ref[(it + 1) % 2]
                mx = jnp.full((8, TQ), -jnp.inf, f32)
            l = jnp.zeros((8, TQ), f32)
            acc = jnp.zeros((DH, TQ), f32)
            for cidx in range(NC):
                rows = pl.ds(cidx * CK, CK)
                p = jnp.exp2(s_ref[rows, :] - m_cur)
                l = l + red8(p, jnp.sum)
                acc = acc + jnp.dot(vt_ref[hrow, rows], p.astype(bf16),
                                    preferred_element_type=f32)
                if with_next:
                    sn = jnp.dot(k_ref[gn, rows, :], qmn, preferred_element_type=f32)
                    s_ref[rows, :] = sn
                    mx = jnp.maximum(mx, red8(sn, jnp.max))
            lsum = jnp.sum(l, axis=0, keepdims=True)
            ot_ref[j, hrow, :] = (acc / lsum).astype(bf16)
            if with_next:
                qm_ref[it % 2] = qmask(jnp.minimum(it + 2, n_items - 1))[1]
                return jnp.max(mx, axis=0, keepdims=True)

        m_last = lax.fori_loop(0, n_items - 1, lambda it, m: attend(it, m, True), m0)
        attend(n_items - 1, m_last, False)

        cp_wmb.wait()
        cp_wo.wait()
        cp_w1.wait()
        cp_w2.wait()
        mod_b = jnp.dot(sc, wmod_ref[:, 2 * D:6 * D], preferred_element_type=f32)
        ga = mod_b[:, 0 * D:1 * D]
        sb = mod_b[:, 1 * D:2 * D]
        cb = mod_b[:, 2 * D:3 * D]
        gb = mod_b[:, 3 * D:4 * D]
        b1 = b1_ref[...].astype(f32).reshape(1, F)
        b2 = b2_ref[...].astype(f32).reshape(1, D)

        def mlp_body(r, carry):
            rows = pl.ds(pl.multiple_of(r * TR, TR), TR)
            attn = lax.dot_general(ot_ref[r], wo_ref[...],
                                   (((0,), (0,)), ((), ())),
                                   preferred_element_type=f32)
            x1 = x_ref[rows, :].astype(f32) + ga * attn
            h2 = (layernorm(x1) * (1.0 + cb) + sb).astype(bf16)
            a = jnp.dot(h2, w1_ref[...], preferred_element_type=f32) + b1
            a = jnp.maximum(a, 0.0)
            a = (a * a).astype(bf16)
            y = jnp.dot(a, w2_ref[...], preferred_element_type=f32) + b2
            o_ref[rows, :] = (x1 + gb * y).astype(o_ref.dtype)
            pltpu.make_async_copy(o_ref.at[rows, :], o_hbm.at[rows, :], out_sems.at[r]).start()
            return carry

        lax.fori_loop(0, S // TR, mlp_body, 0)
        for r in range(S // TR):
            pltpu.make_async_copy(o_ref.at[pl.ds(r * TR, TR), :], o_hbm.at[pl.ds(r * TR, TR), :],
                                  out_sems.at[r]).wait()

    any_spec = pl.BlockSpec(memory_space=pl.ANY)
    vmem_spec = pl.BlockSpec(memory_space=pltpu.VMEM)
    out = pl.pallas_call(
        kernel,
        out_shape=jax.ShapeDtypeStruct((S, D), A_x.dtype),
        in_specs=[any_spec, any_spec, any_spec, any_spec, vmem_spec, any_spec,
                  vmem_spec, vmem_spec, any_spec],
        out_specs=any_spec,
        scratch_shapes=[
            pltpu.VMEM((S, D), bf16),
            pltpu.VMEM((D, 3 * D), bf16),
            pltpu.VMEM((D, D), bf16),
            pltpu.VMEM((D, F), bf16),
            pltpu.VMEM((F, D), bf16),
            pltpu.VMEM((D, 6 * D), bf16),
            pltpu.VMEM((S, D), bf16),
            pltpu.VMEM((2, LANES, TQ), bf16),
            pltpu.VMEM((G, S, LANES), bf16),
            pltpu.VMEM((G, NQ, LANES, TQ), bf16),
            pltpu.VMEM((D, S), bf16),
            pltpu.VMEM((NQ, D, TQ), bf16),
            pltpu.VMEM((S, TQ), f32),
            pltpu.SemaphoreType.DMA((1 + NQ + 7,)),
            pltpu.SemaphoreType.DMA((S // TR,)),
        ],
        compiler_params=pltpu.CompilerParams(vmem_limit_bytes=100 * 1024 * 1024),
    )(
        A_x.reshape(S, D), A_wqkv, A_wo, B_w1, B_b1, B_w2,
        B_b2, c, w_mod,
    )
    return out.reshape(B, S, D)
```

```python
import jax
import jax.numpy as jnp
from jax import lax
import jax.experimental.pallas as pl
import jax.experimental.pallas.tpu as pltpu

_LOG2E = 1.4426950408889634
_EPS = 1e-05


@jax.jit
def pallas_adaLN_cond__mha_block__dense_activation_squared_relu__prompt_kernel(
    A_x: jax.Array,
    A_wqkv: jax.Array,
    A_wo: jax.Array,
    B_x: jax.Array,
    B_w1: jax.Array,
    B_b1: jax.Array,
    B_w2: jax.Array,
    B_b2: jax.Array,
    c: jax.Array,
    w_mod: jax.Array,
):
    del B_x
    B, S, D = A_x.shape
    assert B == 1
    H = 32
    DH = D // H
    F = B_w1.shape[1]
    LANES = 128
    HPG = LANES // DH
    G = D // LANES
    TQ = 512
    CK = 128
    NQ = S // TQ
    NC = S // CK
    TR = TQ
    q_scale = (DH ** -0.5) * _LOG2E

    f32 = jnp.float32
    bf16 = jnp.bfloat16

    def layernorm(x):
        m = jnp.mean(x, axis=-1, keepdims=True)
        xc = x - m
        v = jnp.mean(xc * xc, axis=-1, keepdims=True)
        return xc * lax.rsqrt(v + _EPS)

    def kernel(x_hbm, wqkv_hbm, wo_hbm, w1_hbm, b1_ref, w2_hbm, b2_ref, c_ref,
               wmod_hbm, o_hbm,
               x_ref, wqkv_ref, wo_ref, w1_ref, w2_ref, wmod_ref, o_ref,
               qm_ref, k_ref, qt_ref, vt_ref, ot_ref, s_ref, in_sems, out_sems):
        cp_wma = pltpu.make_async_copy(wmod_hbm.at[:, 0:2 * D], wmod_ref.at[:, 0:2 * D], in_sems.at[0])
        cp_x = [pltpu.make_async_copy(x_hbm.at[pl.ds(r * TQ, TQ), :], x_ref.at[pl.ds(r * TQ, TQ), :],
                                      in_sems.at[1 + r]) for r in range(NQ)]
        base = 1 + NQ
        cp_wk = pltpu.make_async_copy(wqkv_hbm.at[:, D:2 * D], wqkv_ref.at[:, D:2 * D], in_sems.at[base])
        cp_wq = pltpu.make_async_copy(wqkv_hbm.at[:, 0:D], wqkv_ref.at[:, 0:D], in_sems.at[base + 1])
        cp_wv = pltpu.make_async_copy(wqkv_hbm.at[:, 2 * D:3 * D], wqkv_ref.at[:, 2 * D:3 * D], in_sems.at[base + 2])
        cp_wmb = pltpu.make_async_copy(wmod_hbm.at[:, 2 * D:6 * D], wmod_ref.at[:, 2 * D:6 * D], in_sems.at[base + 3])
        cp_wo = pltpu.make_async_copy(wo_hbm, wo_ref, in_sems.at[base + 4])
        cp_w1 = pltpu.make_async_copy(w1_hbm, w1_ref, in_sems.at[base + 5])
        cp_w2 = pltpu.make_async_copy(w2_hbm, w2_ref, in_sems.at[base + 6])
        cp_wma.start()
        cp_x[0].start()
        cp_wk.start()
        cp_wq.start()
        cp_wv.start()
        for r in range(1, NQ):
            cp_x[r].start()

        cc = c_ref[...].astype(f32)
        sc = (cc * jax.nn.sigmoid(cc)).astype(bf16)
        cp_wma.wait()
        mod_a = jnp.dot(sc, wmod_ref[:, 0:2 * D], preferred_element_type=f32)
        sa = mod_a[:, 0 * D:1 * D]
        ca = mod_a[:, 1 * D:2 * D]

        def proj_body(r, carry, first=False):
            rows = pl.ds(pl.multiple_of(r * TQ, TQ), TQ)
            pltpu.make_async_copy(x_hbm.at[rows, :], x_ref.at[rows, :], in_sems.at[1 + r]).wait()
            xr = x_ref[rows, :].astype(f32)
            h = (layernorm(xr) * (1.0 + ca) + sa).astype(bf16)
            if first:
                cp_wk.wait()
            kk = jnp.dot(h, wqkv_ref[:, D:2 * D], preferred_element_type=f32)
            for g in range(G):
                k_ref[g, rows, :] = kk[:, g * LANES:(g + 1) * LANES].astype(bf16)
            if first:
                cp_wq.wait()
            qt = lax.dot_general(wqkv_ref[:, 0:D], h, (((0,), (1,)), ((), ())),
                                 preferred_element_type=f32)
            qt = (qt * q_scale).astype(bf16)
            for g in range(G):
                qt_ref[g, r] = qt[g * LANES:(g + 1) * LANES, :]
            if first:
                cp_wv.wait()
            vt = lax.dot_general(wqkv_ref[:, 2 * D:3 * D], h, (((0,), (1,)), ((), ())),
                                 preferred_element_type=f32)
            vt_ref[:, rows] = vt.astype(bf16)
            return carry

        proj_body(0, 0, first=True)
        lax.fori_loop(1, NQ, proj_body, 0)

        cp_wmb.start()
        cp_wo.start()
        cp_w1.start()
        cp_w2.start()

        n_items = H * NQ

        def qmask(it):
            h = it // NQ
            j = it % NQ
            g = h // HPG
            hh = h % HPG
            q = qt_ref[g, j]
            row = lax.broadcasted_iota(jnp.int32, q.shape, 0)
            keep = (row >= hh * DH) & (row < hh * DH + DH)
            return g, jnp.where(keep, q, jnp.zeros_like(q))

        def red8(x, op):
            return op(x.reshape(CK // 8, 8, TQ), axis=0)

        g0, qm0 = qmask(0)
        mx0 = jnp.full((8, TQ), -jnp.inf, f32)
        for cidx in range(NC):
            rows = pl.ds(cidx * CK, CK)
            sn = jnp.dot(k_ref[g0, rows, :], qm0, preferred_element_type=f32)
            s_ref[rows, :] = sn
            mx0 = jnp.maximum(mx0, red8(sn, jnp.max))
        m0 = jnp.max(mx0, axis=0, keepdims=True)
        qm_ref[1] = qmask(1)[1]

        def attend(it, m_cur, with_next):
            h = it // NQ
            j = it % NQ
            hrow = pl.ds(pl.multiple_of(h * DH, DH), DH)
            if with_next:
                gn = ((it + 1) // NQ) // HPG
                qmn = qm_ref[(it + 1) % 2]
                mx = jnp.full((8, TQ), -jnp.inf, f32)
            l = jnp.zeros((8, TQ), f32)
            acc = jnp.zeros((DH, TQ), f32)
            for cidx in range(NC):
                rows = pl.ds(cidx * CK, CK)
                p = jnp.exp2(s_ref[rows, :] - m_cur)
                l = l + red8(p, jnp.sum)
                acc = acc + jnp.dot(vt_ref[hrow, rows], p.astype(bf16),
                                    preferred_element_type=f32)
                if with_next:
                    sn = jnp.dot(k_ref[gn, rows, :], qmn, preferred_element_type=f32)
                    s_ref[rows, :] = sn
                    mx = jnp.maximum(mx, red8(sn, jnp.max))
            lsum = jnp.sum(l, axis=0, keepdims=True)
            ot_ref[j, hrow, :] = (acc / lsum).astype(bf16)
            if with_next:
                qm_ref[it % 2] = qmask(jnp.minimum(it + 2, n_items - 1))[1]
                return jnp.max(mx, axis=0, keepdims=True)

        m_last = lax.fori_loop(0, n_items - 1, lambda it, m: attend(it, m, True), m0)
        attend(n_items - 1, m_last, False)

        cp_wmb.wait()
        cp_wo.wait()
        cp_w1.wait()
        cp_w2.wait()
        mod_b = jnp.dot(sc, wmod_ref[:, 2 * D:6 * D], preferred_element_type=f32)
        ga = mod_b[:, 0 * D:1 * D]
        sb = mod_b[:, 1 * D:2 * D]
        cb = mod_b[:, 2 * D:3 * D]
        gb = mod_b[:, 3 * D:4 * D]
        b1 = b1_ref[...].astype(f32).reshape(1, F)
        b2 = b2_ref[...].astype(f32).reshape(1, D)

        def mlp_body(r, carry):
            rows = pl.ds(pl.multiple_of(r * TR, TR), TR)
            attn = lax.dot_general(ot_ref[r], wo_ref[...],
                                   (((0,), (0,)), ((), ())),
                                   preferred_element_type=f32)
            x1 = x_ref[rows, :].astype(f32) + ga * attn
            h2 = (layernorm(x1) * (1.0 + cb) + sb).astype(bf16)
            a = jnp.dot(h2, w1_ref[...], preferred_element_type=f32) + b1
            a = jnp.maximum(a, 0.0)
            a = (a * a).astype(bf16)
            y = jnp.dot(a, w2_ref[...], preferred_element_type=f32) + b2
            o_ref[rows, :] = (x1 + gb * y).astype(o_ref.dtype)
            pltpu.make_async_copy(o_ref.at[rows, :], o_hbm.at[rows, :], out_sems.at[r]).start()
            return carry

        lax.fori_loop(0, S // TR, mlp_body, 0)
        for r in range(S // TR):
            pltpu.make_async_copy(o_ref.at[pl.ds(r * TR, TR), :], o_hbm.at[pl.ds(r * TR, TR), :],
                                  out_sems.at[r]).wait()

    any_spec = pl.BlockSpec(memory_space=pl.ANY)
    vmem_spec = pl.BlockSpec(memory_space=pltpu.VMEM)
    out = pl.pallas_call(
        kernel,
        out_shape=jax.ShapeDtypeStruct((S, D), A_x.dtype),
        in_specs=[any_spec, any_spec, any_spec, any_spec, vmem_spec, any_spec,
                  vmem_spec, vmem_spec, any_spec],
        out_specs=any_spec,
        scratch_shapes=[
            pltpu.VMEM((S, D), bf16),
            pltpu.VMEM((D, 3 * D), bf16),
            pltpu.VMEM((D, D), bf16),
            pltpu.VMEM((D, F), bf16),
            pltpu.VMEM((F, D), bf16),
            pltpu.VMEM((D, 6 * D), bf16),
            pltpu.VMEM((S, D), bf16),
            pltpu.VMEM((2, LANES, TQ), bf16),
            pltpu.VMEM((G, S, LANES), bf16),
            pltpu.VMEM((G, NQ, LANES, TQ), bf16),
            pltpu.VMEM((D, S), bf16),
            pltpu.VMEM((NQ, D, TQ), bf16),
            pltpu.VMEM((S, TQ), f32),
            pltpu.SemaphoreType.DMA((1 + NQ + 7,)),
            pltpu.SemaphoreType.DMA((S // TR,)),
        ],
        compiler_params=pltpu.CompilerParams(vmem_limit_bytes=100 * 1024 * 1024),
    )(
        A_x.reshape(S, D), A_wqkv, A_wo, B_w1, B_b1, B_w2,
        B_b2, c, w_mod,
    )
    return out.reshape(B, S, D)
```

```python
import jax
import jax.numpy as jnp
from jax import lax
import jax.experimental.pallas as pl
import jax.experimental.pallas.tpu as pltpu

_LOG2E = 1.4426950408889634
_EPS = 1e-05


@jax.jit
def pallas_adaLN_cond__mha_block__dense_activation_squared_relu__prompt_kernel(
    A_x: jax.Array,
    A_wqkv: jax.Array,
    A_wo: jax.Array,
    B_x: jax.Array,
    B_w1: jax.Array,
    B_b1: jax.Array,
    B_w2: jax.Array,
    B_b2: jax.Array,
    c: jax.Array,
    w_mod: jax.Array,
):
    del B_x
    B, S, D = A_x.shape
    assert B == 1
    H = 32
    DH = D // H
    F = B_w1.shape[1]
    LANES = 128
    HPG = LANES // DH
    G = D // LANES
    TQ = 512
    CK = 128
    NQ = S // TQ
    NC = S // CK
    TR = TQ
    q_scale = (DH ** -0.5) * _LOG2E

    f32 = jnp.float32
    bf16 = jnp.bfloat16

    def layernorm(x):
        m = jnp.mean(x, axis=-1, keepdims=True)
        xc = x - m
        v = jnp.mean(xc * xc, axis=-1, keepdims=True)
        return xc * lax.rsqrt(v + _EPS)

    def kernel(x_hbm, wqkv_hbm, wo_hbm, w1_hbm, b1_ref, w2_hbm, b2_ref, c_ref,
               wmod_hbm, o_hbm,
               x_ref, wqkv_ref, wo_ref, w1_ref, w2_ref, wmod_ref, o_ref,
               qm_ref, k_ref, qt_ref, vt_ref, ot_ref, s_ref, p_ref, in_sems, out_sems):
        cp_wma = pltpu.make_async_copy(wmod_hbm.at[:, 0:2 * D], wmod_ref.at[:, 0:2 * D], in_sems.at[0])
        cp_x = [pltpu.make_async_copy(x_hbm.at[pl.ds(r * TQ, TQ), :], x_ref.at[pl.ds(r * TQ, TQ), :],
                                      in_sems.at[1 + r]) for r in range(NQ)]
        base = 1 + NQ
        cp_wk = pltpu.make_async_copy(wqkv_hbm.at[:, D:2 * D], wqkv_ref.at[:, D:2 * D], in_sems.at[base])
        cp_wq = pltpu.make_async_copy(wqkv_hbm.at[:, 0:D], wqkv_ref.at[:, 0:D], in_sems.at[base + 1])
        cp_wv = pltpu.make_async_copy(wqkv_hbm.at[:, 2 * D:3 * D], wqkv_ref.at[:, 2 * D:3 * D], in_sems.at[base + 2])
        cp_wmb = pltpu.make_async_copy(wmod_hbm.at[:, 2 * D:6 * D], wmod_ref.at[:, 2 * D:6 * D], in_sems.at[base + 3])
        cp_wo = pltpu.make_async_copy(wo_hbm, wo_ref, in_sems.at[base + 4])
        cp_w1 = pltpu.make_async_copy(w1_hbm, w1_ref, in_sems.at[base + 5])
        cp_w2 = pltpu.make_async_copy(w2_hbm, w2_ref, in_sems.at[base + 6])
        cp_wma.start()
        cp_x[0].start()
        cp_wk.start()
        cp_wq.start()
        cp_wv.start()
        for r in range(1, NQ):
            cp_x[r].start()

        cc = c_ref[...].astype(f32)
        sc = (cc * jax.nn.sigmoid(cc)).astype(bf16)
        cp_wma.wait()
        mod_a = jnp.dot(sc, wmod_ref[:, 0:2 * D], preferred_element_type=f32)
        sa = mod_a[:, 0 * D:1 * D]
        ca = mod_a[:, 1 * D:2 * D]

        def proj_body(r, carry, first=False):
            rows = pl.ds(pl.multiple_of(r * TQ, TQ), TQ)
            pltpu.make_async_copy(x_hbm.at[rows, :], x_ref.at[rows, :], in_sems.at[1 + r]).wait()
            xr = x_ref[rows, :].astype(f32)
            h = (layernorm(xr) * (1.0 + ca) + sa).astype(bf16)
            if first:
                cp_wk.wait()
            kk = jnp.dot(h, wqkv_ref[:, D:2 * D], preferred_element_type=f32)
            for g in range(G):
                k_ref[g, rows, :] = kk[:, g * LANES:(g + 1) * LANES].astype(bf16)
            if first:
                cp_wq.wait()
            qt = lax.dot_general(wqkv_ref[:, 0:D], h, (((0,), (1,)), ((), ())),
                                 preferred_element_type=f32)
            qt = (qt * q_scale).astype(bf16)
            for g in range(G):
                qt_ref[g, r] = qt[g * LANES:(g + 1) * LANES, :]
            if first:
                cp_wv.wait()
            vt = lax.dot_general(wqkv_ref[:, 2 * D:3 * D], h, (((0,), (1,)), ((), ())),
                                 preferred_element_type=f32)
            vt_ref[:, rows] = vt.astype(bf16)
            return carry

        proj_body(0, 0, first=True)
        lax.fori_loop(1, NQ, proj_body, 0)

        cp_wmb.start()
        cp_wo.start()
        cp_w1.start()
        cp_w2.start()

        n_items = H * NQ

        def qmask(it):
            h = it // NQ
            j = it % NQ
            g = h // HPG
            hh = h % HPG
            q = qt_ref[g, j]
            row = lax.broadcasted_iota(jnp.int32, q.shape, 0)
            keep = (row >= hh * DH) & (row < hh * DH + DH)
            return g, jnp.where(keep, q, jnp.zeros_like(q))

        def red8(x, op):
            return op(x.reshape(CK // 8, 8, TQ), axis=0)

        def step(it, m_cur, l_prev, do_pv, do_exp, do_qk, staged_q):
            if do_qk:
                if staged_q:
                    gn = ((it + 1) // NQ) // HPG
                    qmn = qm_ref[(it + 1) % 2]
                else:
                    gn, qmn = qmask(it + 1)
                mx = jnp.full((8, TQ), -jnp.inf, f32)
            if do_exp:
                l = jnp.zeros((8, TQ), f32)
            if do_pv:
                hp = (it - 1) // NQ
                jp = (it - 1) % NQ
                hrow = pl.ds(pl.multiple_of(hp * DH, DH), DH)
                acc = jnp.zeros((DH, TQ), f32)
            for cidx in range(NC):
                rows = pl.ds(cidx * CK, CK)
                if do_pv:
                    acc = acc + jnp.dot(vt_ref[hrow, rows], p_ref[rows, :],
                                        preferred_element_type=f32)
                if do_exp:
                    p = jnp.exp2(s_ref[rows, :] - m_cur)
                    l = l + red8(p, jnp.sum)
                    p_ref[rows, :] = p.astype(bf16)
                if do_qk:
                    sn = jnp.dot(k_ref[gn, rows, :], qmn, preferred_element_type=f32)
                    s_ref[rows, :] = sn
                    mx = jnp.maximum(mx, red8(sn, jnp.max))
            if do_pv:
                ot_ref[jp, hrow, :] = (acc / l_prev).astype(bf16)
            if do_qk:
                qm_ref[it % 2] = qmask(jnp.minimum(it + 2, n_items - 1))[1]
            m_next = jnp.max(mx, axis=0, keepdims=True) if do_qk else m_cur
            l_out = jnp.sum(l, axis=0, keepdims=True) if do_exp else l_prev
            return m_next, l_out

        zrow = jnp.zeros((1, TQ), f32)
        ml = step(-1, zrow, zrow, False, False, True, False)
        ml = step(0, ml[0], ml[1], False, True, True, True)
        ml = lax.fori_loop(
            1, n_items - 1,
            lambda it, c: step(it, c[0], c[1], True, True, True, True), ml)
        ml = step(n_items - 1, ml[0], ml[1], True, True, False, False)
        step(n_items, ml[0], ml[1], True, False, False, False)

        cp_wmb.wait()
        cp_wo.wait()
        cp_w1.wait()
        cp_w2.wait()
        mod_b = jnp.dot(sc, wmod_ref[:, 2 * D:6 * D], preferred_element_type=f32)
        ga = mod_b[:, 0 * D:1 * D]
        sb = mod_b[:, 1 * D:2 * D]
        cb = mod_b[:, 2 * D:3 * D]
        gb = mod_b[:, 3 * D:4 * D]
        b1 = b1_ref[...].astype(f32).reshape(1, F)
        b2 = b2_ref[...].astype(f32).reshape(1, D)

        def mlp_body(r, carry):
            rows = pl.ds(pl.multiple_of(r * TR, TR), TR)
            attn = lax.dot_general(ot_ref[r], wo_ref[...],
                                   (((0,), (0,)), ((), ())),
                                   preferred_element_type=f32)
            x1 = x_ref[rows, :].astype(f32) + ga * attn
            h2 = (layernorm(x1) * (1.0 + cb) + sb).astype(bf16)
            a = jnp.dot(h2, w1_ref[...], preferred_element_type=f32) + b1
            a = jnp.maximum(a, 0.0)
            a = (a * a).astype(bf16)
            y = jnp.dot(a, w2_ref[...], preferred_element_type=f32) + b2
            o_ref[rows, :] = (x1 + gb * y).astype(o_ref.dtype)
            pltpu.make_async_copy(o_ref.at[rows, :], o_hbm.at[rows, :], out_sems.at[r]).start()
            return carry

        lax.fori_loop(0, S // TR, mlp_body, 0)
        for r in range(S // TR):
            pltpu.make_async_copy(o_ref.at[pl.ds(r * TR, TR), :], o_hbm.at[pl.ds(r * TR, TR), :],
                                  out_sems.at[r]).wait()

    any_spec = pl.BlockSpec(memory_space=pl.ANY)
    vmem_spec = pl.BlockSpec(memory_space=pltpu.VMEM)
    out = pl.pallas_call(
        kernel,
        out_shape=jax.ShapeDtypeStruct((S, D), A_x.dtype),
        in_specs=[any_spec, any_spec, any_spec, any_spec, vmem_spec, any_spec,
                  vmem_spec, vmem_spec, any_spec],
        out_specs=any_spec,
        scratch_shapes=[
            pltpu.VMEM((S, D), bf16),
            pltpu.VMEM((D, 3 * D), bf16),
            pltpu.VMEM((D, D), bf16),
            pltpu.VMEM((D, F), bf16),
            pltpu.VMEM((F, D), bf16),
            pltpu.VMEM((D, 6 * D), bf16),
            pltpu.VMEM((S, D), bf16),
            pltpu.VMEM((2, LANES, TQ), bf16),
            pltpu.VMEM((G, S, LANES), bf16),
            pltpu.VMEM((G, NQ, LANES, TQ), bf16),
            pltpu.VMEM((D, S), bf16),
            pltpu.VMEM((NQ, D, TQ), bf16),
            pltpu.VMEM((S, TQ), f32),
            pltpu.VMEM((S, TQ), bf16),
            pltpu.SemaphoreType.DMA((1 + NQ + 7,)),
            pltpu.SemaphoreType.DMA((S // TR,)),
        ],
        compiler_params=pltpu.CompilerParams(vmem_limit_bytes=100 * 1024 * 1024),
    )(
        A_x.reshape(S, D), A_wqkv, A_wo, B_w1, B_b1, B_w2,
        B_b2, c, w_mod,
    )
    return out.reshape(B, S, D)
```

```python
import jax
import jax.numpy as jnp
from jax import lax
import jax.experimental.pallas as pl
import jax.experimental.pallas.tpu as pltpu

_LOG2E = 1.4426950408889634
_EPS = 1e-05


@jax.jit
def pallas_adaLN_cond__mha_block__dense_activation_squared_relu__prompt_kernel(
    A_x: jax.Array,
    A_wqkv: jax.Array,
    A_wo: jax.Array,
    B_x: jax.Array,
    B_w1: jax.Array,
    B_b1: jax.Array,
    B_w2: jax.Array,
    B_b2: jax.Array,
    c: jax.Array,
    w_mod: jax.Array,
):
    del B_x
    B, S, D = A_x.shape
    assert B == 1
    H = 32
    DH = D // H
    F = B_w1.shape[1]
    LANES = 128
    HPG = LANES // DH
    G = D // LANES
    TQ = 512
    CK = 128
    NQ = S // TQ
    NC = S // CK
    TR = TQ
    q_scale = (DH ** -0.5) * _LOG2E

    f32 = jnp.float32
    bf16 = jnp.bfloat16

    def layernorm(x):
        m = jnp.mean(x, axis=-1, keepdims=True)
        xc = x - m
        v = jnp.mean(xc * xc, axis=-1, keepdims=True)
        return xc * lax.rsqrt(v + _EPS)

    def kernel(x_hbm, wqkv_hbm, wo_hbm, w1_hbm, b1_ref, w2_hbm, b2_ref, c_ref,
               wmod_hbm, o_hbm,
               x_ref, wqkv_ref, wo_ref, w1_ref, w2_ref, wmod_ref, o_ref,
               qm_ref, k_ref, qt_ref, vt_ref, ot_ref, s_ref, p_ref, in_sems, out_sems):
        cp_wma = pltpu.make_async_copy(wmod_hbm.at[:, 0:2 * D], wmod_ref.at[:, 0:2 * D], in_sems.at[0])
        cp_x = [pltpu.make_async_copy(x_hbm.at[pl.ds(r * TQ, TQ), :], x_ref.at[pl.ds(r * TQ, TQ), :],
                                      in_sems.at[1 + r]) for r in range(NQ)]
        base = 1 + NQ
        cp_wk = pltpu.make_async_copy(wqkv_hbm.at[:, D:2 * D], wqkv_ref.at[:, D:2 * D], in_sems.at[base])
        cp_wq = pltpu.make_async_copy(wqkv_hbm.at[:, 0:D], wqkv_ref.at[:, 0:D], in_sems.at[base + 1])
        cp_wv = pltpu.make_async_copy(wqkv_hbm.at[:, 2 * D:3 * D], wqkv_ref.at[:, 2 * D:3 * D], in_sems.at[base + 2])
        cp_wmb = pltpu.make_async_copy(wmod_hbm.at[:, 2 * D:6 * D], wmod_ref.at[:, 2 * D:6 * D], in_sems.at[base + 3])
        cp_wo = pltpu.make_async_copy(wo_hbm, wo_ref, in_sems.at[base + 4])
        cp_w1 = pltpu.make_async_copy(w1_hbm, w1_ref, in_sems.at[base + 5])
        cp_w2 = pltpu.make_async_copy(w2_hbm, w2_ref, in_sems.at[base + 6])
        cp_wma.start()
        cp_x[0].start()
        cp_wk.start()
        cp_wq.start()
        cp_wv.start()
        for r in range(1, NQ):
            cp_x[r].start()

        cc = c_ref[...].astype(f32)
        sc = (cc * jax.nn.sigmoid(cc)).astype(bf16)
        cp_wma.wait()
        mod_a = jnp.dot(sc, wmod_ref[:, 0:2 * D], preferred_element_type=f32)
        sa = mod_a[:, 0 * D:1 * D]
        ca = mod_a[:, 1 * D:2 * D]

        def proj_body(r, carry, first=False):
            rows = pl.ds(pl.multiple_of(r * TQ, TQ), TQ)
            pltpu.make_async_copy(x_hbm.at[rows, :], x_ref.at[rows, :], in_sems.at[1 + r]).wait()
            xr = x_ref[rows, :].astype(f32)
            h = (layernorm(xr) * (1.0 + ca) + sa).astype(bf16)
            if first:
                cp_wk.wait()
            kk = jnp.dot(h, wqkv_ref[:, D:2 * D], preferred_element_type=f32)
            for g in range(G):
                k_ref[g, rows, :] = kk[:, g * LANES:(g + 1) * LANES].astype(bf16)
            if first:
                cp_wq.wait()
            qt = lax.dot_general(wqkv_ref[:, 0:D], h, (((0,), (1,)), ((), ())),
                                 preferred_element_type=f32)
            qt = (qt * q_scale).astype(bf16)
            for g in range(G):
                qt_ref[g, r] = qt[g * LANES:(g + 1) * LANES, :]
            if first:
                cp_wv.wait()
            vt = lax.dot_general(wqkv_ref[:, 2 * D:3 * D], h, (((0,), (1,)), ((), ())),
                                 preferred_element_type=f32)
            vt_ref[:, rows] = vt.astype(bf16)
            return carry

        proj_body(0, 0, first=True)
        lax.fori_loop(1, NQ, proj_body, 0)

        cp_wmb.start()
        cp_wo.start()
        cp_w1.start()
        cp_w2.start()

        n_items = H * NQ

        def qmask(it):
            h = it // NQ
            j = it % NQ
            g = h // HPG
            hh = h % HPG
            q = qt_ref[g, j]
            row = lax.broadcasted_iota(jnp.int32, q.shape, 0)
            keep = (row >= hh * DH) & (row < hh * DH + DH)
            return g, jnp.where(keep, q, jnp.zeros_like(q))

        def red8(x, op):
            return op(x.reshape(CK // 8, 8, TQ), axis=0)

        def step(it, m_cur, l_prev, do_pv, do_exp, do_qk, staged_q):
            if do_qk:
                if staged_q:
                    gn = ((it + 1) // NQ) // HPG
                    qmn = qm_ref[(it + 1) % 2]
                else:
                    gn, qmn = qmask(it + 1)
                mx = jnp.full((8, TQ), -jnp.inf, f32)
            if do_exp:
                l = jnp.zeros((8, TQ), f32)
            if do_pv:
                hp = (it - 1) // NQ
                jp = (it - 1) % NQ
                hrow = pl.ds(pl.multiple_of(hp * DH, DH), DH)
                acc = jnp.zeros((DH, TQ), f32)
            for cidx in range(NC):
                rows = pl.ds(cidx * CK, CK)
                if do_pv:
                    acc = acc + jnp.dot(vt_ref[hrow, rows], p_ref[rows, :],
                                        preferred_element_type=f32)
                if do_exp:
                    p = jnp.exp2(s_ref[rows, :] - m_cur)
                    l = l + red8(p, jnp.sum)
                    p_ref[rows, :] = p.astype(bf16)
                if do_qk:
                    sn = jnp.dot(k_ref[gn, rows, :], qmn, preferred_element_type=f32)
                    s_ref[rows, :] = sn
                    mx = jnp.maximum(mx, red8(sn, jnp.max))
            if do_pv:
                ot_ref[jp, hrow, :] = (acc / l_prev).astype(bf16)
            if do_qk:
                qm_ref[it % 2] = qmask(jnp.minimum(it + 2, n_items - 1))[1]
            m_next = jnp.max(mx, axis=0, keepdims=True) if do_qk else m_cur
            l_out = jnp.sum(l, axis=0, keepdims=True) if do_exp else l_prev
            return m_next, l_out

        zrow = jnp.zeros((1, TQ), f32)
        ml = step(-1, zrow, zrow, False, False, True, False)
        ml = step(0, ml[0], ml[1], False, True, True, True)
        ml = lax.fori_loop(
            1, n_items - 1,
            lambda it, c: step(it, c[0], c[1], True, True, True, True), ml)
        ml = step(n_items - 1, ml[0], ml[1], True, True, False, False)
        step(n_items, ml[0], ml[1], True, False, False, False)

        cp_wmb.wait()
        cp_wo.wait()
        cp_w1.wait()
        cp_w2.wait()
        mod_b = jnp.dot(sc, wmod_ref[:, 2 * D:6 * D], preferred_element_type=f32)
        ga = mod_b[:, 0 * D:1 * D]
        sb = mod_b[:, 1 * D:2 * D]
        cb = mod_b[:, 2 * D:3 * D]
        gb = mod_b[:, 3 * D:4 * D]
        b1 = b1_ref[...].astype(f32).reshape(1, F)
        b2 = b2_ref[...].astype(f32).reshape(1, D)

        HM = TR // 2

        def mlp_body(r, carry):
            x1s, h2s = [], []
            for u in range(2):
                rows = pl.ds(pl.multiple_of(r * TR + u * HM, HM), HM)
                attn = lax.dot_general(ot_ref[r, :, u * HM:(u + 1) * HM], wo_ref[...],
                                       (((0,), (0,)), ((), ())),
                                       preferred_element_type=f32)
                x1 = x_ref[rows, :].astype(f32) + ga * attn
                x1s.append(x1)
                h2s.append((layernorm(x1) * (1.0 + cb) + sb).astype(bf16))
            for u in range(2):
                rows = pl.ds(pl.multiple_of(r * TR + u * HM, HM), HM)
                a = jnp.dot(h2s[u], w1_ref[...], preferred_element_type=f32) + b1
                a = jnp.maximum(a, 0.0)
                a = (a * a).astype(bf16)
                y = jnp.dot(a, w2_ref[...], preferred_element_type=f32) + b2
                o_ref[rows, :] = (x1s[u] + gb * y).astype(o_ref.dtype)
            rows = pl.ds(pl.multiple_of(r * TR, TR), TR)
            pltpu.make_async_copy(o_ref.at[rows, :], o_hbm.at[rows, :], out_sems.at[r]).start()
            return carry

        lax.fori_loop(0, S // TR, mlp_body, 0)
        for r in range(S // TR):
            pltpu.make_async_copy(o_ref.at[pl.ds(r * TR, TR), :], o_hbm.at[pl.ds(r * TR, TR), :],
                                  out_sems.at[r]).wait()

    any_spec = pl.BlockSpec(memory_space=pl.ANY)
    vmem_spec = pl.BlockSpec(memory_space=pltpu.VMEM)
    out = pl.pallas_call(
        kernel,
        out_shape=jax.ShapeDtypeStruct((S, D), A_x.dtype),
        in_specs=[any_spec, any_spec, any_spec, any_spec, vmem_spec, any_spec,
                  vmem_spec, vmem_spec, any_spec],
        out_specs=any_spec,
        scratch_shapes=[
            pltpu.VMEM((S, D), bf16),
            pltpu.VMEM((D, 3 * D), bf16),
            pltpu.VMEM((D, D), bf16),
            pltpu.VMEM((D, F), bf16),
            pltpu.VMEM((F, D), bf16),
            pltpu.VMEM((D, 6 * D), bf16),
            pltpu.VMEM((S, D), bf16),
            pltpu.VMEM((2, LANES, TQ), bf16),
            pltpu.VMEM((G, S, LANES), bf16),
            pltpu.VMEM((G, NQ, LANES, TQ), bf16),
            pltpu.VMEM((D, S), bf16),
            pltpu.VMEM((NQ, D, TQ), bf16),
            pltpu.VMEM((S, TQ), f32),
            pltpu.VMEM((S, TQ), bf16),
            pltpu.SemaphoreType.DMA((1 + NQ + 7,)),
            pltpu.SemaphoreType.DMA((S // TR,)),
        ],
        compiler_params=pltpu.CompilerParams(vmem_limit_bytes=100 * 1024 * 1024),
    )(
        A_x.reshape(S, D), A_wqkv, A_wo, B_w1, B_b1, B_w2,
        B_b2, c, w_mod,
    )
    return out.reshape(B, S, D)
```

```python
import jax
import jax.numpy as jnp
from jax import lax
import jax.experimental.pallas as pl
import jax.experimental.pallas.tpu as pltpu

_LOG2E = 1.4426950408889634
_EPS = 1e-05


@jax.jit
def pallas_adaLN_cond__mha_block__dense_activation_squared_relu__prompt_kernel(
    A_x: jax.Array,
    A_wqkv: jax.Array,
    A_wo: jax.Array,
    B_x: jax.Array,
    B_w1: jax.Array,
    B_b1: jax.Array,
    B_w2: jax.Array,
    B_b2: jax.Array,
    c: jax.Array,
    w_mod: jax.Array,
):
    del B_x
    B, S, D = A_x.shape
    assert B == 1
    H = 32
    DH = D // H
    F = B_w1.shape[1]
    LANES = 128
    HPG = LANES // DH
    G = D // LANES
    TQ = 512
    CK = 128
    NQ = S // TQ
    NC = S // CK
    TR = TQ
    q_scale = (DH ** -0.5) * _LOG2E

    f32 = jnp.float32
    bf16 = jnp.bfloat16

    def layernorm(x):
        m = jnp.mean(x, axis=-1, keepdims=True)
        xc = x - m
        v = jnp.mean(xc * xc, axis=-1, keepdims=True)
        return xc * lax.rsqrt(v + _EPS)

    def kernel(x_hbm, wqkv_hbm, wo_hbm, w1_hbm, b1_ref, w2_hbm, b2_ref, c_ref,
               wmod_hbm, o_hbm,
               x_ref, wqkv_ref, wo_ref, w1_ref, w2_ref, wmod_ref, o_ref,
               qm_ref, k_ref, qt_ref, vt_ref, ot_ref, s_ref, p_ref, in_sems, out_sems):
        cp_wma = pltpu.make_async_copy(wmod_hbm.at[:, 0:2 * D], wmod_ref.at[:, 0:2 * D], in_sems.at[0])
        cp_x = [pltpu.make_async_copy(x_hbm.at[pl.ds(r * TQ, TQ), :], x_ref.at[pl.ds(r * TQ, TQ), :],
                                      in_sems.at[1 + r]) for r in range(NQ)]
        base = 1 + NQ
        cp_wk = pltpu.make_async_copy(wqkv_hbm.at[:, D:2 * D], wqkv_ref.at[:, D:2 * D], in_sems.at[base])
        cp_wq = pltpu.make_async_copy(wqkv_hbm.at[:, 0:D], wqkv_ref.at[:, 0:D], in_sems.at[base + 1])
        cp_wv = pltpu.make_async_copy(wqkv_hbm.at[:, 2 * D:3 * D], wqkv_ref.at[:, 2 * D:3 * D], in_sems.at[base + 2])
        cp_wmb = pltpu.make_async_copy(wmod_hbm.at[:, 2 * D:6 * D], wmod_ref.at[:, 2 * D:6 * D], in_sems.at[base + 3])
        cp_wo = pltpu.make_async_copy(wo_hbm, wo_ref, in_sems.at[base + 4])
        cp_w1 = pltpu.make_async_copy(w1_hbm, w1_ref, in_sems.at[base + 5])
        cp_w2 = pltpu.make_async_copy(w2_hbm, w2_ref, in_sems.at[base + 6])
        cp_wma.start()
        cp_x[0].start()
        cp_wk.start()
        cp_wq.start()
        cp_wv.start()
        for r in range(1, NQ):
            cp_x[r].start()

        cc = c_ref[...].astype(f32)
        sc = (cc * jax.nn.sigmoid(cc)).astype(bf16)
        cp_wma.wait()
        mod_a = jnp.dot(sc, wmod_ref[:, 0:2 * D], preferred_element_type=f32)
        sa = mod_a[:, 0 * D:1 * D]
        ca = mod_a[:, 1 * D:2 * D]

        def proj_body(r, carry, first=False):
            rows = pl.ds(pl.multiple_of(r * TQ, TQ), TQ)
            pltpu.make_async_copy(x_hbm.at[rows, :], x_ref.at[rows, :], in_sems.at[1 + r]).wait()
            hs = []
            for u in range(2):
                hrows = pl.ds(pl.multiple_of(r * TQ + u * (TQ // 2), TQ // 2), TQ // 2)
                xr = x_ref[hrows, :].astype(f32)
                hu = (layernorm(xr) * (1.0 + ca) + sa).astype(bf16)
                hs.append(hu)
                if first and u == 0:
                    cp_wk.wait()
                kk = jnp.dot(hu, wqkv_ref[:, D:2 * D], preferred_element_type=f32)
                for g in range(G):
                    k_ref[g, hrows, :] = kk[:, g * LANES:(g + 1) * LANES].astype(bf16)
            h = jnp.concatenate(hs, axis=0)
            if first:
                cp_wq.wait()
            qt = lax.dot_general(wqkv_ref[:, 0:D], h, (((0,), (1,)), ((), ())),
                                 preferred_element_type=f32)
            qt = (qt * q_scale).astype(bf16)
            for g in range(G):
                qt_ref[g, r] = qt[g * LANES:(g + 1) * LANES, :]
            if first:
                cp_wv.wait()
            vt = lax.dot_general(wqkv_ref[:, 2 * D:3 * D], h, (((0,), (1,)), ((), ())),
                                 preferred_element_type=f32)
            vt_ref[:, rows] = vt.astype(bf16)
            return carry

        proj_body(0, 0, first=True)
        lax.fori_loop(1, NQ, proj_body, 0)

        cp_wmb.start()
        cp_wo.start()
        cp_w1.start()
        cp_w2.start()

        n_items = H * NQ

        def qmask(it):
            h = it // NQ
            j = it % NQ
            g = h // HPG
            hh = h % HPG
            q = qt_ref[g, j]
            row = lax.broadcasted_iota(jnp.int32, q.shape, 0)
            keep = (row >= hh * DH) & (row < hh * DH + DH)
            return g, jnp.where(keep, q, jnp.zeros_like(q))

        def red8(x, op):
            return op(x.reshape(CK // 8, 8, TQ), axis=0)

        def step(it, m_cur, l_prev, do_pv, do_exp, do_qk, staged_q):
            if do_qk:
                if staged_q:
                    gn = ((it + 1) // NQ) // HPG
                    qmn = qm_ref[(it + 1) % 2]
                else:
                    gn, qmn = qmask(it + 1)
                mx = jnp.full((8, TQ), -jnp.inf, f32)
            if do_exp:
                l = jnp.zeros((8, TQ), f32)
            if do_pv:
                hp = (it - 1) // NQ
                jp = (it - 1) % NQ
                hrow = pl.ds(pl.multiple_of(hp * DH, DH), DH)
                acc = jnp.zeros((DH, TQ), f32)
            for cidx in range(NC):
                rows = pl.ds(cidx * CK, CK)
                if do_pv:
                    acc = acc + jnp.dot(vt_ref[hrow, rows], p_ref[rows, :],
                                        preferred_element_type=f32)
                if do_exp:
                    p = jnp.exp2(s_ref[rows, :] - m_cur)
                    l = l + red8(p, jnp.sum)
                    p_ref[rows, :] = p.astype(bf16)
                if do_qk:
                    sn = jnp.dot(k_ref[gn, rows, :], qmn, preferred_element_type=f32)
                    s_ref[rows, :] = sn
                    mx = jnp.maximum(mx, red8(sn, jnp.max))
            if do_pv:
                ot_ref[jp, hrow, :] = (acc / l_prev).astype(bf16)
            if do_qk:
                qm_ref[it % 2] = qmask(jnp.minimum(it + 2, n_items - 1))[1]
            m_next = jnp.max(mx, axis=0, keepdims=True) if do_qk else m_cur
            l_out = jnp.sum(l, axis=0, keepdims=True) if do_exp else l_prev
            return m_next, l_out

        zrow = jnp.zeros((1, TQ), f32)
        ml = step(-1, zrow, zrow, False, False, True, False)
        ml = step(0, ml[0], ml[1], False, True, True, True)
        ml = lax.fori_loop(
            1, n_items - 1,
            lambda it, c: step(it, c[0], c[1], True, True, True, True), ml)
        ml = step(n_items - 1, ml[0], ml[1], True, True, False, False)
        step(n_items, ml[0], ml[1], True, False, False, False)

        cp_wmb.wait()
        cp_wo.wait()
        cp_w1.wait()
        cp_w2.wait()
        mod_b = jnp.dot(sc, wmod_ref[:, 2 * D:6 * D], preferred_element_type=f32)
        ga = mod_b[:, 0 * D:1 * D]
        sb = mod_b[:, 1 * D:2 * D]
        cb = mod_b[:, 2 * D:3 * D]
        gb = mod_b[:, 3 * D:4 * D]
        b1 = b1_ref[...].astype(f32).reshape(1, F)
        b2 = b2_ref[...].astype(f32).reshape(1, D)

        NH = 4
        HM = TR // NH

        def mlp_body(r, carry):
            x1s, h2s = [], []
            for u in range(NH):
                rows = pl.ds(pl.multiple_of(r * TR + u * HM, HM), HM)
                attn = lax.dot_general(ot_ref[r, :, u * HM:(u + 1) * HM], wo_ref[...],
                                       (((0,), (0,)), ((), ())),
                                       preferred_element_type=f32)
                x1 = x_ref[rows, :].astype(f32) + ga * attn
                x1s.append(x1)
                h2s.append((layernorm(x1) * (1.0 + cb) + sb).astype(bf16))
            for u in range(NH):
                rows = pl.ds(pl.multiple_of(r * TR + u * HM, HM), HM)
                a = jnp.dot(h2s[u], w1_ref[...], preferred_element_type=f32) + b1
                a = jnp.maximum(a, 0.0)
                a = (a * a).astype(bf16)
                y = jnp.dot(a, w2_ref[...], preferred_element_type=f32) + b2
                o_ref[rows, :] = (x1s[u] + gb * y).astype(o_ref.dtype)
            rows = pl.ds(pl.multiple_of(r * TR, TR), TR)
            pltpu.make_async_copy(o_ref.at[rows, :], o_hbm.at[rows, :], out_sems.at[r]).start()
            return carry

        lax.fori_loop(0, S // TR, mlp_body, 0)
        for r in range(S // TR):
            pltpu.make_async_copy(o_ref.at[pl.ds(r * TR, TR), :], o_hbm.at[pl.ds(r * TR, TR), :],
                                  out_sems.at[r]).wait()

    any_spec = pl.BlockSpec(memory_space=pl.ANY)
    vmem_spec = pl.BlockSpec(memory_space=pltpu.VMEM)
    out = pl.pallas_call(
        kernel,
        out_shape=jax.ShapeDtypeStruct((S, D), A_x.dtype),
        in_specs=[any_spec, any_spec, any_spec, any_spec, vmem_spec, any_spec,
                  vmem_spec, vmem_spec, any_spec],
        out_specs=any_spec,
        scratch_shapes=[
            pltpu.VMEM((S, D), bf16),
            pltpu.VMEM((D, 3 * D), bf16),
            pltpu.VMEM((D, D), bf16),
            pltpu.VMEM((D, F), bf16),
            pltpu.VMEM((F, D), bf16),
            pltpu.VMEM((D, 6 * D), bf16),
            pltpu.VMEM((S, D), bf16),
            pltpu.VMEM((2, LANES, TQ), bf16),
            pltpu.VMEM((G, S, LANES), bf16),
            pltpu.VMEM((G, NQ, LANES, TQ), bf16),
            pltpu.VMEM((D, S), bf16),
            pltpu.VMEM((NQ, D, TQ), bf16),
            pltpu.VMEM((S, TQ), f32),
            pltpu.VMEM((S, TQ), bf16),
            pltpu.SemaphoreType.DMA((1 + NQ + 7,)),
            pltpu.SemaphoreType.DMA((S // TR,)),
        ],
        compiler_params=pltpu.CompilerParams(vmem_limit_bytes=100 * 1024 * 1024),
    )(
        A_x.reshape(S, D), A_wqkv, A_wo, B_w1, B_b1, B_w2,
        B_b2, c, w_mod,
    )
    return out.reshape(B, S, D)
```
